```python
import jax
import jax.numpy as jnp

def _softmax(x, axis=-1):
    return jax.nn.softmax(x, axis=axis)

def _gelu(x):
    return jax.nn.gelu(x, approximate=True)

def _silu(x):
    return jax.nn.silu(x)

def _sigmoid(x):
    return jax.nn.sigmoid(x)

def _layernorm(x, axis=-1, eps=1e-05):
    m = jnp.mean(x, axis=axis, keepdims=True)
    v = jnp.var(x, axis=axis, keepdims=True)
    return (x - m) / jnp.sqrt(v + eps)

def _scatter_add(tgt, idx, src, axis=0):
    return tgt.at[idx].add(src)

def _segment_sum(src, seg, n):
    return jax.ops.segment_sum(src, seg, n)

class _Rng:

    def __init__(self, key):
        self._k = key

    def _next(self):
        self._k, sub = jax.random.split(self._k)
        return sub

    def normal(self, shape):
        return jax.random.normal(self._next(), shape, dtype=jnp.bfloat16)

    def randint(self, lo, hi, shape):
        return jax.random.randint(self._next(), shape, lo, hi, dtype=jnp.int32)

    def uniform(self, shape, lo=0.0, hi=1.0):
        return jax.random.uniform(self._next(), shape, jnp.bfloat16, lo, hi)

    def permutation(self, n):
        return jax.random.permutation(self._next(), n)
kernel_name = 'adaLN_cond__compressed_kv_cla__moe_arch_mod__prompt'

def setup_inputs():
    _rng = _Rng(jax.random.key(int.from_bytes(__import__("os").urandom(4), "little")))
    _w = lambda a: (lambda t: t.astype(jnp.bfloat16) if jnp.issubdtype(t.dtype, jnp.floating) else t)(jnp.asarray(a))

    def _A_setup():
        B, H, Sq, Sk, D, M = (1, 32, 2048, 2048, 128, 640)
        Dc = 4 * D
        return {'x': _w((lambda *s: _rng.normal(s) * 0.05)(B, Sq, M)), 'c_kv': _w((lambda *s: _rng.normal(s) * 0.05)(B, Sk, Dc)), 'w_q': _w((lambda *s: _rng.normal(s) * 0.05)(M, H, D) * M ** (-0.5)), 'w_uk': _w((lambda *s: _rng.normal(s) * 0.05)(Dc, H, D) * Dc ** (-0.5)), 'w_uv': _w((lambda *s: _rng.normal(s) * 0.05)(Dc, H, D) * Dc ** (-0.5)), 'w_o': _w((lambda *s: _rng.normal(s) * 0.05)(H, D, M) * (H * D) ** (-0.5))}
    _A_in = _A_setup()

    def _B_setup():
        B, S, D, F, C = (1, 2048, 640, 1728, 8)
        return {'x': _w((lambda *s: _rng.normal(s) * 0.05)(B, S, D)), 'w_r': _w((lambda *s: _rng.normal(s) * 0.05)(D)), 'w_gate': _w((lambda *s: _rng.normal(s) * 0.05)(D, F)), 'w_up': _w((lambda *s: _rng.normal(s) * 0.05)(D, F)), 'w_down': _w((lambda *s: _rng.normal(s) * 0.05)(F, D))}
    _B_in = _B_setup()
    return {'A_x': _A_in['x'], 'A_c_kv': _A_in['c_kv'], 'A_w_q': _A_in['w_q'], 'A_w_uk': _A_in['w_uk'], 'A_w_uv': _A_in['w_uv'], 'A_w_o': _A_in['w_o'], 'B_x': _B_in['x'], 'B_w_r': _B_in['w_r'], 'B_w_gate': _B_in['w_gate'], 'B_w_up': _B_in['w_up'], 'B_w_down': _B_in['w_down'], 'c': _w((lambda *s: _rng.normal(s) * 0.05)(1, 640)), 'w_mod': _w((lambda *s: _rng.normal(s) * 0.05)(640, 6 * 640) * 640 ** (-0.5))}

def reference(A_x, A_c_kv, A_w_q, A_w_uk, A_w_uv, A_w_o, B_x, B_w_r, B_w_gate, B_w_up, B_w_down, c, w_mod):

    def _A_ref(x, c_kv, w_q, w_uk, w_uv, w_o):
        B, Sq, M = (x.shape[0], x.shape[1], x.shape[2])
        Sk = c_kv.shape[1]
        H, D = (w_q.shape[1], w_q.shape[2])
        q = jnp.einsum('bqm,mhd->bhqd', x, w_q)
        k = jnp.einsum('bkc,chd->bhkd', c_kv, w_uk)
        v = jnp.einsum('bkc,chd->bhkd', c_kv, w_uv)
        scores = jnp.einsum('bhqd,bhkd->bhqk', q, k) * D ** (-0.5)
        off = Sk - Sq
        qi = jnp.arange(Sq)[:, None]
        kj = jnp.arange(Sk)[None, :]
        cmask = kj <= qi + off
        scores = jnp.where(cmask[None, None], scores, -1000000000.0)
        p = _softmax(scores, axis=-1)
        ctx = jnp.einsum('bhqk,bhkd->bhqd', p, v)
        return jnp.einsum('bhqd,hdm->bqm', ctx, w_o)

    def _B_ref(x, w_r, w_gate, w_up, w_down):
        B, S, D = x.shape
        C = 8
        r = x @ w_r
        idx = jnp.argsort(-r, axis=-1)[:, :C]
        idx_e = jnp.repeat(idx.reshape(B, C, 1), D, axis=2)
        x_sel = jnp.take_along_axis(x, idx_e, axis=1)
        g = _silu(x_sel @ w_gate)
        u = x_sel @ w_up
        y = g * u @ w_down
        r_sel = _sigmoid(jnp.take_along_axis(r, idx, axis=1))
        y = y * r_sel.reshape(B, C, 1)
        b_off = (jnp.arange(B) * S).reshape(B, 1)
        flat_idx = (idx + b_off).reshape(B * C)
        zero = (x * 0.0).reshape(B * S, D)
        upd = _scatter_add(zero, flat_idx, y.reshape(B * C, D), axis=0)
        return x + upd.reshape(B, S, D)
    x = A_x
    mod = (_silu(c) @ w_mod).reshape(c.shape[0], 6, 1, -1)
    sa, ca, ga, sb, cb, gb = (mod[:, 0].copy(), mod[:, 1].copy(), mod[:, 2].copy(), mod[:, 3].copy(), mod[:, 4].copy(), mod[:, 5].copy())
    h = _layernorm(x, axis=-1) * (1 + ca) + sa
    x = x + ga * _A_ref(h, A_c_kv, A_w_q, A_w_uk, A_w_uv, A_w_o)
    h = _layernorm(x, axis=-1) * (1 + cb) + sb
    x = x + gb * _B_ref(h, B_w_r, B_w_gate, B_w_up, B_w_down)
    return x
```

```python
import math

import jax
import jax.numpy as jnp
from jax import lax
import jax.experimental.pallas as pl
import jax.experimental.pallas.tpu as pltpu

F32 = jnp.float32
BF16 = jnp.bfloat16
U32 = jnp.uint32
I32 = jnp.int32

_NT = (((1,), (1,)), ((), ()))
_TOPC = 8
_EPS = 1e-5
_LOG2E = math.log2(math.e)
_MASKED = -1000000000.0 * _LOG2E
_BQ = 256


def _rb(v):
    return v.astype(BF16).astype(F32)


def _pack(v):
    return pltpu.bitcast(v.astype(BF16), U32)


def _rows(ref, a, b):
    return pltpu.bitcast(ref[a // 2:b // 2, :], BF16)


def _layernorm(x):
    n = x.shape[-1]
    mean = jnp.sum(x, axis=-1, keepdims=True) * (1.0 / n)
    d = x - mean
    var = jnp.sum(d * d, axis=-1, keepdims=True) * (1.0 / n)
    den = _rb(jnp.sqrt(_rb(_rb(var) + _EPS)))
    return _rb(_rb(x - _rb(mean)) * (1.0 / den))


def _kernel(x_hbm, ckv_hbm, wq_hbm, wuk_hbm, wuv_hbm, wo_hbm, wr_ref, wg_hbm,
            wu_hbm, wd_hbm, c_ref, wmod_hbm, out_hbm,
            x_v, ckv_v, wmod_v, w_v, wo_v, wg_v, wu_v, wd_v,
            h_s, ckv_s, q_s, k_s, v_s, ctx_s, x1_v, h2_v, out_v,
            in_sem, w_sem, out_sem, fix_sem):
    S, M = x_v.shape
    DC = ckv_v.shape[1]
    H, _, D = ctx_s.shape
    bq = _BQ
    nb = S // bq
    T = bq // 128
    q_scale = (D ** -0.5) * _LOG2E

    def w_copies(j):
        return (
            pltpu.make_async_copy(wuk_hbm.bitcast(U32).at[:, j, :],
                                  w_v.at[j, pl.ds(M, DC), :], w_sem.at[j]),
            pltpu.make_async_copy(wuv_hbm.bitcast(U32).at[:, j, :],
                                  w_v.at[j, pl.ds(M + DC, DC), :], w_sem.at[j]),
            pltpu.make_async_copy(wq_hbm.bitcast(U32).at[:, j, :],
                                  w_v.at[j, pl.ds(0, M), :], w_sem.at[j]),
        )

    cp_ckv = pltpu.make_async_copy(ckv_hbm, ckv_v, in_sem.at[0])
    cp_mod_a = pltpu.make_async_copy(wmod_hbm.at[:, pl.ds(0, 2 * M)],
                                     wmod_v.at[:, pl.ds(0, 2 * M)], in_sem.at[1])
    cp_x = pltpu.make_async_copy(x_hbm, x_v, in_sem.at[2])
    cp_mod_b = pltpu.make_async_copy(wmod_hbm.at[:, pl.ds(2 * M, 4 * M)],
                                     wmod_v.at[:, pl.ds(2 * M, 4 * M)], in_sem.at[3])
    cp_wo = pltpu.make_async_copy(wo_hbm, wo_v, in_sem.at[4])
    cp_wg = pltpu.make_async_copy(wg_hbm, wg_v, in_sem.at[5])
    cp_wu = pltpu.make_async_copy(wu_hbm, wu_v, in_sem.at[6])
    cp_wd = pltpu.make_async_copy(wd_hbm, wd_v, in_sem.at[7])

    def out_copy(i):
        return pltpu.make_async_copy(out_v.at[pl.ds(i * bq, bq), :],
                                     out_hbm.at[pl.ds(i * bq, bq), :], out_sem.at[i])

    def head_weights(n):
        shift = jnp.asarray(16 - 16 * (n % 2), U32)

        def half(a, b):
            w = w_v[n // 2, a:b, :]
            return pltpu.bitcast((w << shift) & U32(0xFFFF0000), F32)

        wq = half(0, M).astype(BF16)
        wkv = jnp.concatenate([half(M, M + DC), half(M + DC, M + 2 * DC)],
                              axis=1).astype(BF16)
        return wq, wkv

    def proj_kv(wkv, a, b):
        kv = jnp.dot(_rows(ckv_s, a, b), wkv, preferred_element_type=F32)
        k_s[a // 2:b // 2, :] = _pack(kv[:, :D])
        v_s[a // 2:b // 2, :] = _pack(kv[:, D:])

    def proj_q(wq, a, b):
        q = jnp.dot(_rows(h_s, a, b), wq, preferred_element_type=F32)
        q_s[a // 2:b // 2, :] = _pack(q * q_scale)

    def attention(n, after_block):
        tri = (lax.broadcasted_iota(I32, (128, 128), 1)
               <= lax.broadcasted_iota(I32, (128, 128), 0))
        live = {}

        def scores(i):
            l0 = i * bq + 128
            s = lax.dot_general(_rows(q_s, i * bq, (i + 1) * bq), _rows(k_s, 0, l0),
                                _NT, preferred_element_type=F32)
            extra = [
                lax.dot_general(_rows(q_s, i * bq + u * 128, (i + 1) * bq),
                                _rows(k_s, l0 + (u - 1) * 128, l0 + u * 128),
                                _NT, preferred_element_type=F32)
                for u in range(1, T)
            ]
            for t in range(T):
                tiles = [s[t * 128:(t + 1) * 128, j * 128:(j + 1) * 128]
                         for j in range(l0 // 128)]
                tiles += [extra[u - 1][(t - u) * 128:(t - u + 1) * 128]
                          for u in range(1, t + 1)]
                tiles[-1] = jnp.where(tri, tiles[-1], _MASKED)
                mx = tiles[0]
                for tile in tiles[1:]:
                    mx = jnp.maximum(mx, tile)
                live[i, t] = (tiles, jnp.max(mx, axis=1, keepdims=True))

        def values(i):
            ps, invs = [], []
            for t in range(T):
                tiles, m = live.pop((i, t))
                pt = [jnp.exp2(tile - m) for tile in tiles]
                l = pt[0]
                for p in pt[1:]:
                    l = l + p
                ps.append(pt)
                invs.append(1.0 / jnp.sum(l, axis=1, keepdims=True))
            l0 = i * bq + 128
            n0 = l0 // 128
            p = jnp.concatenate(
                [jnp.concatenate(ps[t][:n0], axis=1) for t in range(T)], axis=0)
            o = jnp.dot(p.astype(BF16), _rows(v_s, 0, l0), preferred_element_type=F32)
            extra = [
                jnp.dot(jnp.concatenate([ps[t][n0 + u - 1] for t in range(u, T)],
                                        axis=0).astype(BF16),
                        _rows(v_s, l0 + (u - 1) * 128, l0 + u * 128),
                        preferred_element_type=F32)
                for u in range(1, T)
            ]
            for t in range(T):
                ot = o[t * 128:(t + 1) * 128]
                for u in range(1, t + 1):
                    ot = ot + extra[u - 1][(t - u) * 128:(t - u + 1) * 128]
                r0 = (i * bq + t * 128) // 2
                ctx_s[n, r0:r0 + 64, :] = _pack(ot * invs[t])

        scores(nb - 1)
        for i in reversed(range(nb)):
            if i > 0:
                scores(i - 1)
            values(i)
            after_block(i)

    for cp in w_copies(0):
        cp.start()
    cp_ckv.start()
    cp_mod_a.start()
    cp_x.start()

    cf = c_ref[...].astype(F32)
    silu_c = jnp.broadcast_to(cf * jax.nn.sigmoid(cf), (16, M)).astype(BF16)

    for cp in w_copies(0):
        cp.wait()
    cp_ckv.wait()
    wq0, wkv0 = head_weights(0)
    ckv_s[...] = pltpu.bitcast(ckv_v[...], U32)
    proj_kv(wkv0, 0, S)

    cp_mod_a.wait()
    mod_a = _rb(jnp.dot(silu_c, wmod_v[:, :2 * M], preferred_element_type=F32)[:1])
    sa, ca1 = mod_a[:, :M], _rb(1.0 + mod_a[:, M:])
    cp_x.wait()

    def start_rest(j, carry):
        for cp in w_copies(j):
            cp.start()
        return carry

    lax.fori_loop(1, H // 2, start_rest, 0)
    for cp in (cp_mod_b, cp_wo, cp_wg, cp_wu, cp_wd):
        cp.start()

    for i in range(nb):
        a, b = i * bq, (i + 1) * bq
        xf = x_v[a:b, :].astype(F32)
        mean = jnp.sum(xf, axis=-1, keepdims=True) * (1.0 / M)
        d = xf - mean
        var = jnp.sum(d * d, axis=-1, keepdims=True) * (1.0 / M)
        h_s[a // 2:b // 2, :] = _pack(d * lax.rsqrt(var + _EPS) * ca1 + sa)
        proj_q(wq0, a, b)

    def head_step(n, carry):
        @pl.when(n % 2 == 1)
        def _():
            for cp in w_copies((n + 1) // 2):
                cp.wait()

        wq, wkv = head_weights(n + 1)

        def project_next(i):
            proj_kv(wkv, i * bq, (i + 1) * bq)
            proj_q(wq, i * bq, (i + 1) * bq)

        attention(n, project_next)
        return carry

    lax.fori_loop(0, H - 1, head_step, 0)

    for cp in (cp_mod_b, cp_wo, cp_wg, cp_wu, cp_wd):
        cp.wait()
    mod_b = _rb(jnp.dot(silu_c, wmod_v[:, 2 * M:], preferred_element_type=F32)[:1])
    ga, sb = mod_b[:, :M], mod_b[:, M:2 * M]
    cb1, gb = _rb(1.0 + mod_b[:, 2 * M:3 * M]), mod_b[:, 3 * M:]

    wr = wr_ref[...].astype(F32)
    wr = jnp.concatenate([wr[j:j + 1, :] for j in range(M // 128)], axis=1)
    wr = jnp.broadcast_to(wr, (S // 128, M)).astype(BF16)
    tile_id = lax.broadcasted_iota(I32, (S // 128, 128), 0)
    router = [jnp.zeros((S // 128, 128), F32)]

    def finish_block(i):
        a, b = i * bq, (i + 1) * bq
        ctx = jnp.concatenate(
            [pltpu.bitcast(ctx_s[n, a // 2:b // 2, :], BF16) for n in range(H)], axis=1)
        att = _rb(jnp.dot(ctx, wo_v[...], preferred_element_type=F32))
        x1b = (x_v[a:b, :].astype(F32) + _rb(ga * att)).astype(BF16)
        x1 = x1b.astype(F32)
        h2b = (_rb(_layernorm(x1) * cb1) + sb).astype(BF16)
        h2 = h2b.astype(F32)
        x1_v[a:b, :] = x1b
        h2_v[a:b, :] = h2b
        out_v[a:b, :] = (x1 + _rb(gb * (h2 + h2 * 0.0))).astype(BF16)
        out_copy(i).start()
        r = lax.dot_general(wr, h2b, _NT, preferred_element_type=F32)
        for t in range(T):
            router[0] = jnp.where(tile_id == i * T + t, r[:, t * 128:(t + 1) * 128],
                                  router[0])

    attention(H - 1, finish_block)

    r = _rb(router[0]) + 0.0
    bits = lax.shift_right_logical(pltpu.bitcast(r, I32), 16)
    order = jnp.where(bits >= 0x8000, 0xFFFF - bits, bits + 0x8000)
    order = jnp.where(r == 0.0, 0x8000, order)
    order = jnp.where(r != r, 0, order)
    token = tile_id * 128 + lax.broadcasted_iota(I32, (S // 128, 128), 1)
    key = pltpu.bitcast(0x20000000 + order * S + (S - 1 - token), F32)

    sub = lax.broadcasted_iota(I32, (16, M), 0)
    picks = []
    x_sel = jnp.zeros((16, M), F32)
    x1_sel = jnp.zeros((16, M), F32)
    r_sel = jnp.zeros((16, 1), F32)
    for s in range(_TOPC):
        top = jnp.max(jnp.max(key, axis=0, keepdims=True), axis=1, keepdims=True)
        hit = key == top
        key = jnp.where(hit, 0.0, key)
        r_top = jnp.sum(jnp.sum(jnp.where(hit, r, 0.0), axis=0, keepdims=True),
                        axis=1, keepdims=True)
        idx = (S - 1) - (pltpu.bitcast(top, I32)[0, 0] & (S - 1))
        base = pl.multiple_of(idx & -16, 16)
        here = sub == (idx & 15)
        picks.append((base, here))

        def row(ref):
            v = jnp.where(here, ref[pl.ds(base, 16), :].astype(F32), 0.0)
            return jnp.sum(v, axis=0, keepdims=True)

        x_sel = jnp.where(sub == s, row(h2_v), x_sel)
        x1_sel = jnp.where(sub == s, row(x1_v), x1_sel)
        r_sel = jnp.where(sub[:, :1] == s, r_top, r_sel)

    xb = x_sel.astype(BF16)
    g = _rb(lax.dot_general(xb, wg_v[...], _NT, preferred_element_type=F32))
    u = _rb(lax.dot_general(xb, wu_v[...], _NT, preferred_element_type=F32))
    gu = (_rb(g * jax.nn.sigmoid(g)) * u).astype(BF16)
    y = _rb(jnp.dot(gu, wd_v[...], preferred_element_type=F32))
    y = _rb(y * _rb(jax.nn.sigmoid(r_sel)))
    fixed = x1_sel + _rb(gb * _rb(x_sel + (x_sel * 0.0 + y)))

    for i in range(nb):
        out_copy(i).wait()
    for s, (base, here) in enumerate(picks):
        old = out_v[pl.ds(base, 16), :].astype(F32)
        out_v[pl.ds(base, 16), :] = jnp.where(here, fixed[s:s + 1, :], old).astype(BF16)

    def fix_copy(s):
        base = picks[s][0]
        return pltpu.make_async_copy(out_v.at[pl.ds(base, 16), :],
                                     out_hbm.at[pl.ds(base, 16), :], fix_sem.at[s])

    first = []
    for s in range(_TOPC):
        f = jnp.bool_(True)
        for e in range(s):
            f = jnp.logical_and(f, picks[e][0] != picks[s][0])
        first.append(f)
    for s in range(_TOPC):
        pl.when(first[s])(fix_copy(s).start)
    for s in range(_TOPC):
        pl.when(first[s])(fix_copy(s).wait)


@jax.jit
def pallas_adaLN_cond__compressed_kv_cla__moe_arch_mod__prompt_kernel(
    A_x: jax.Array,
    A_c_kv: jax.Array,
    A_w_q: jax.Array,
    A_w_uk: jax.Array,
    A_w_uv: jax.Array,
    A_w_o: jax.Array,
    B_x: jax.Array,
    B_w_r: jax.Array,
    B_w_gate: jax.Array,
    B_w_up: jax.Array,
    B_w_down: jax.Array,
    c: jax.Array,
    w_mod: jax.Array,
):
    del B_x
    B, S, M = A_x.shape
    DC = A_c_kv.shape[-1]
    _, H, D = A_w_q.shape
    F = B_w_down.shape[0]
    assert B == 1 and A_c_kv.shape[1] == S and D == 128
    assert S % _BQ == 0 and S & (S - 1) == 0 and S <= 4096 and H % 2 == 0

    hbm = pl.BlockSpec(memory_space=pl.ANY)
    vmem = pl.BlockSpec(memory_space=pltpu.VMEM)
    out = pl.pallas_call(
        _kernel,
        out_shape=jax.ShapeDtypeStruct((S, M), BF16),
        in_specs=[hbm, hbm, hbm, hbm, hbm, hbm, vmem, hbm, hbm, hbm, vmem, hbm],
        out_specs=hbm,
        scratch_shapes=[
            pltpu.VMEM((S, M), BF16),
            pltpu.VMEM((S, DC), BF16),
            pltpu.VMEM((M, 6 * M), BF16),
            pltpu.VMEM((H // 2, M + 2 * DC, D), U32),
            pltpu.VMEM((H * D, M), BF16),
            pltpu.VMEM((F, M), BF16),
            pltpu.VMEM((F, M), BF16),
            pltpu.VMEM((F, M), BF16),
            pltpu.VMEM((S // 2, M), U32),
            pltpu.VMEM((S // 2, DC), U32),
            pltpu.VMEM((S // 2, D), U32),
            pltpu.VMEM((S // 2, D), U32),
            pltpu.VMEM((S // 2, D), U32),
            pltpu.VMEM((H, S // 2, D), U32),
            pltpu.VMEM((S, M), BF16),
            pltpu.VMEM((S, M), BF16),
            pltpu.VMEM((S, M), BF16),
            pltpu.SemaphoreType.DMA((8,)),
            pltpu.SemaphoreType.DMA((H // 2,)),
            pltpu.SemaphoreType.DMA((S // _BQ,)),
            pltpu.SemaphoreType.DMA((_TOPC,)),
        ],
        compiler_params=pltpu.CompilerParams(vmem_limit_bytes=110 * 1024 * 1024),
        name="adaln_mla_mod",
    )(
        A_x.reshape(S, M),
        A_c_kv.reshape(S, DC),
        A_w_q,
        A_w_uk,
        A_w_uv,
        A_w_o.reshape(H * D, M),
        B_w_r.reshape(M // 128, 128),
        B_w_gate.T,
        B_w_up.T,
        B_w_down,
        c,
        w_mod,
    )
    return out.reshape(B, S, M)
```

```python
import math

import jax
import jax.numpy as jnp
import numpy as np
from jax import lax
import jax.experimental.pallas as pl
import jax.experimental.pallas.tpu as pltpu

F32 = jnp.float32
BF16 = jnp.bfloat16
U32 = jnp.uint32
I32 = jnp.int32

_NT = (((1,), (1,)), ((), ()))
_TOPC = 8
_EPS = 1e-5
_LOG2E = math.log2(math.e)
_MASKED = -1000000000.0 * _LOG2E
_BQ = 256
_EARLY = 5
_UNROLL = 2
_MAX_DELAY = 400


def _rb(v):
    return v.astype(BF16).astype(F32)


def _pack(v):
    return pltpu.bitcast(v.astype(BF16), U32)


def _rows(ref, a, b):
    return pltpu.bitcast(ref[a // 2:b // 2, :], BF16)


def _vregs(v):
    return [v[r:r + 8, j:j + 128] for r in range(0, v.shape[0], 8)
            for j in range(0, v.shape[1], 128)]


def _layernorm(x):
    n = x.shape[-1]
    mean = jnp.sum(x, axis=-1, keepdims=True) * (1.0 / n)
    d = x - mean
    var = jnp.sum(d * d, axis=-1, keepdims=True) * (1.0 / n)
    den = _rb(jnp.sqrt(_rb(_rb(var) + _EPS)))
    return _rb(_rb(x - _rb(mean)) * (1.0 / den))


def _plan(steps, pieces):
    busy = [0] * 4
    slots, span = [], {}
    for pos, (name, tile_rows, open_tiles) in enumerate(steps):
        start, end = min(busy), 0
        for j, rows in enumerate(tile_rows):
            mxu = busy.index(min(busy))
            if j in open_tiles:
                slots += [(busy[mxu] + 16 * g, pos, name, j, g) for g in range(rows // 16)]
            busy[mxu] += rows
            end = max(end, busy[mxu])
        span[name] = (pos, start, end)
    plan = {}
    for i, count in enumerate(pieces):
        qk, pv = span["qk", i], span["pv", i]
        free = sorted(s for s in slots
                      if qk[0] < s[1] < pv[0] and qk[2] + _MAX_DELAY <= s[0] < pv[1])
        for piece in range(count if free else 0):
            when = free[0][0] + (free[-1][0] - free[0][0]) * (piece + 1) / count
            _, _, name, j, g = min(free, key=lambda s: abs(s[0] - when))
            plan.setdefault(name, {}).setdefault(j, {}).setdefault(g, []).append((i, piece))
    return plan


def _kernel(x_hbm, ckv_hbm, wq_hbm, wuk_hbm, wuv_hbm, wo_hbm, wr_hbm, wg_hbm,
            wu_hbm, wd_hbm, c_hbm, wmod_hbm, out_hbm,
            x_v, ckv_v, wmod_v, w_v, wo_v, wg_v, wu_v, wd_v, wgu_s, c_v, wr_v,
            h_s, ckv_s, q_s, k_s, v_s, v_early, ctx_s, x1_v, h2_v, out_v, zero_s,
            in_sem, w_sem, out_sem, fix_sem):
    S, M = x_v.shape
    DC = ckv_v.shape[1]
    F, FP = wd_hbm.shape[0], wd_v.shape[0]
    H, _, D = ctx_s.shape
    bq = _BQ
    nb = S // bq
    T = bq // 128
    ncol = M // 128
    q_scale = (D ** -0.5) * _LOG2E
    w_rows = {"q": (0, M), "k": (M, M + DC), "v": (M + DC, M + 2 * DC)}

    def w_copy(kind, j):
        a, b = w_rows[kind]
        src = {"q": wq_hbm, "k": wuk_hbm, "v": wuv_hbm}[kind]
        return pltpu.make_async_copy(src.bitcast(U32).at[:, j, :],
                                     w_v.at[j, pl.ds(a, b - a), :],
                                     w_sem.at["qkv".index(kind) * (H // 2) + j])

    def row_copy(src, dst, sem, start, size):
        return pltpu.make_async_copy(src.at[pl.ds(start, size), :],
                                     dst.at[pl.ds(start, size), :], sem)

    def mod_copy(a, b, sem):
        return pltpu.make_async_copy(wmod_hbm.at[:, pl.ds(a * M, (b - a) * M)],
                                     wmod_v.at[:, pl.ds(a * M, (b - a) * M)], sem)

    cp_early = [w_copy(kind, j) for j in (1, 2) for kind in "qk"]
    cp_main = [w_copy(kind, j) for j in range(3, H // 2)
               for kind in ("qkv" if j < H // 2 - 1 else "qk")]
    cp_late = [
        mod_copy(2, 6, in_sem.at[1]),
        pltpu.make_async_copy(wo_hbm, wo_v, in_sem.at[2]),
        pltpu.make_async_copy(wg_hbm, wg_v.at[pl.ds(0, F), :], in_sem.at[3]),
        pltpu.make_async_copy(wu_hbm, wu_v.at[pl.ds(0, F), :], in_sem.at[4]),
        pltpu.make_async_copy(wd_hbm, wd_v.at[pl.ds(0, F), :], in_sem.at[5]),
        pltpu.make_async_copy(wr_hbm, wr_v, in_sem.at[12]),
    ]

    def after(v, srcs):
        if not srcs:
            return v
        dep = zero_s[...]
        for src in srcs:
            dep = dep & pltpu.bitcast(src, U32)
        dep = jnp.concatenate([dep] * (v.shape[0] // 8), axis=0)
        dep = jnp.concatenate([dep] * (v.shape[1] // 128), axis=1)
        return pltpu.bitcast(pltpu.bitcast(v, U32) | dep, v.dtype)

    plan, partial_sums = {}, {}

    def planned(step, tiles):
        out = list(tiles)
        for j, at in plan.get(step, {}).items():
            per = 16 if out[j].dtype == F32 else 8
            parts, done = [], 0
            for g in sorted(at):
                if done < g * per:
                    parts.append(out[j][done:g * per])
                done = g * per + 8
                parts.append(after(out[j][g * per:done],
                                   [partial_sums[i][piece] for i, piece in at[g]]))
            if done < out[j].shape[0]:
                parts.append(out[j][done:])
            out[j] = jnp.concatenate(parts, axis=0)
        return jnp.concatenate(out, axis=1)

    def key_groups(i):
        return pl.cdiv(i * T + 1, 4)

    def set_plan(steps):
        plan.clear()
        plan.update(_plan(steps, [bq // 8 * key_groups(i) for i in range(nb)]))

    def weight(kind, n):
        a, b = w_rows[kind]
        shift = 16 - 16 * (n & 1)
        shift = np.uint32(shift) if isinstance(n, int) else shift.astype(U32)
        w = (w_v[n >> 1, a:b, :] << shift) & np.uint32(0xFFFF0000)
        return pltpu.bitcast(w, F32).astype(BF16)

    def project(kind, i, w, dst):
        src = h_s if kind == "q" else ckv_s
        rows = slice(i * bq // 2, (i + 1) * bq // 2)
        lhs = planned((kind, i), [src[rows, j:j + 128] for j in range(0, src.shape[1], 128)])
        y = jnp.dot(pltpu.bitcast(lhs, BF16), w, preferred_element_type=F32)
        dst[rows, :] = _pack(y * q_scale if kind == "q" else y)

    def proj_step(kind, i):
        n = (M if kind == "q" else DC) // 128
        return (kind, i), [bq] * n, range(n)

    probs = {}

    def attn_step(kind, i):
        rows = [bq] * (i * T + 1) + [bq - 128 * u for u in range(1, T)]
        return (kind, i), rows, range(0, i * T + 1, 4 if kind == "qk" else 1)

    def scores(i):
        tri = (lax.broadcasted_iota(I32, (128, 128), 1)
               <= lax.broadcasted_iota(I32, (128, 128), 0))
        l0 = i * bq + 128
        q = planned(("qk", i), [q_s[i * bq // 2:(i + 1) * bq // 2, :]] * (l0 // 128))
        q = pltpu.bitcast(q, BF16)
        s = jnp.concatenate(
            [lax.dot_general(q[:, j:j + 128], _rows(k_s, j, min(j + 512, l0)),
                             _NT, preferred_element_type=F32)
             for j in range(0, l0, 512)], axis=1)
        extra = [
            lax.dot_general(_rows(q_s, i * bq + u * 128, (i + 1) * bq),
                            _rows(k_s, l0 + (u - 1) * 128, l0 + u * 128),
                            _NT, preferred_element_type=F32)
            for u in range(1, T)
        ]
        ps, invs, partial_sums[i] = [], [], []
        for t in range(T):
            tiles = [s[t * 128:(t + 1) * 128, j:j + 128] for j in range(0, l0, 128)]
            tiles += [extra[u - 1][(t - u) * 128:(t - u + 1) * 128]
                      for u in range(1, t + 1)]
            tiles[-1] = jnp.where(tri, tiles[-1], _MASKED)
            m = tiles[0]
            for tile in tiles[1:]:
                m = jnp.maximum(m, tile)
            m = jnp.max(m, axis=1, keepdims=True)
            pt = [jnp.exp2(tile - m) for tile in tiles]
            sums = [pt[0]]
            for p in pt[1:]:
                sums.append(sums[-1] + p)
            for g in range(0, 128, 16):
                for k in range(key_groups(i)):
                    part = sums[pl.cdiv(len(pt) * (k + 1), key_groups(i)) - 1]
                    partial_sums[i] += [part[g:g + 8], part[g + 8:g + 16]]
            ps.append(pt)
            invs.append(pltpu.reciprocal(jnp.sum(sums[-1], axis=1, keepdims=True),
                                         full_range=False))
        probs[i] = ps, invs

    def values(n, i, v_ref):
        ps, invs = probs.pop(i)
        l0 = i * bq + 128
        n0 = l0 // 128
        p = planned(("pv", i), [jnp.concatenate([ps[t][j] for t in range(T)], axis=0)
                                for j in range(n0)])
        o = jnp.dot(p.astype(BF16), _rows(v_ref, 0, l0), preferred_element_type=F32)
        extra = [
            jnp.dot(jnp.concatenate([ps[t][n0 + u - 1] for t in range(u, T)],
                                    axis=0).astype(BF16),
                    _rows(v_ref, l0 + (u - 1) * 128, l0 + u * 128),
                    preferred_element_type=F32)
            for u in range(1, T)
        ]
        for t in range(T):
            ot = o[t * 128:(t + 1) * 128]
            for u in range(1, t + 1):
                ot = ot + extra[u - 1][(t - u) * 128:(t - u + 1) * 128]
            r0 = (i * bq + t * 128) // 2
            ctx_s[n, r0:r0 + 64, :] = _pack(ot * invs[t])

    early = list(range(_EARLY)) + [H - 1]

    def ckv_copy(e, a, b):
        return row_copy(ckv_hbm, ckv_v, in_sem.at[6 + e], a * bq, (b - a) * bq)

    def x_copy(e, a, b):
        return row_copy(x_hbm, x_v, in_sem.at[10 + e], a * bq, (b - a) * bq)

    def over(kind, a, b, *heads):
        return [(kind, i, n) for i in range(a, b) for n in heads or (0,)]

    stages = [
        ([ckv_copy(0, 0, 1), w_copy("v", 0)],
         over("ckv", 0, 1) + over("v", 0, 1, 0, 1)),
        ([ckv_copy(1, 1, 2), w_copy("k", 0)],
         over("ckv", 1, 2) + over("v", 1, 2, 0, 1) + over("k", 0, 2)),
        ([ckv_copy(2, 2, 4), w_copy("v", 1)],
         over("ckv", 2, 4) + over("v", 2, 4, 0, 1) + over("k", 2, 4)
         + over("v", 0, 4, 2, 3)),
        ([ckv_copy(3, 4, nb)],
         over("ckv", 4, nb) + over("v", 4, nb, 0, 1) + over("k", 4, nb)
         + over("v", 4, nb, 2, 3)),
        ([mod_copy(0, 2, in_sem.at[0]), pltpu.make_async_copy(c_hbm, c_v, in_sem.at[13]),
          w_copy("q", 0), w_copy("v", 2), x_copy(0, 0, 3)],
         over("mod", 0, 1) + over("norm", 0, 3) + over("v", 0, nb, 4) + over("q", 0, 3)),
        ([w_copy("v", H // 2 - 1), x_copy(1, 3, nb)],
         over("norm", 3, nb) + over("v", 0, nb, H - 1) + over("q", 3, nb)),
    ]
    issue = {0: stages[2][0] + stages[3][0], 1: stages[4][0], 2: stages[5][0],
             5: cp_early + cp_main[:len(cp_main) // 2]}

    for cp in stages[0][0] + stages[1][0]:
        cp.start()
    zero_s[...] = jnp.zeros(zero_s.shape, U32)
    for ref in (wg_v, wu_v, wd_v):
        ref[F:, :] = jnp.zeros((FP - F, M), BF16)
    weights = {}
    for e, (cps, work) in enumerate(stages):
        for cp in cps:
            cp.wait()
        for cp in issue.get(e, []):
            cp.start()
        for kind, i, n in work:
            rows = slice(i * bq, (i + 1) * bq)
            packed = slice(i * bq // 2, (i + 1) * bq // 2)
            if kind == "ckv":
                ckv_s[packed, :] = pltpu.bitcast(ckv_v[rows, :], U32)
            elif kind == "mod":
                cf = c_v[...].astype(F32)
                silu_c = cf * jax.nn.sigmoid(cf)
                mod = _rb(jnp.dot(jnp.broadcast_to(silu_c, (16, M)).astype(BF16),
                                  wmod_v[:, :2 * M], preferred_element_type=F32)[:1])
                sa, ca1 = mod[:, :M], _rb(1.0 + mod[:, M:])
            elif kind == "norm":
                xf = x_v[rows, :].astype(F32)
                d = xf - jnp.sum(xf, axis=-1, keepdims=True) * (1.0 / M)
                var = jnp.sum(d * d, axis=-1, keepdims=True) * (1.0 / M)
                h_s[packed, :] = _pack(d * lax.rsqrt(var + _EPS) * ca1 + sa)
            else:
                if (kind, n) not in weights:
                    weights[kind, n] = weight(kind, n)
                dst = v_early.at[early.index(n)] if kind == "v" else {"q": q_s, "k": k_s}[kind]
                project(kind, i, weights[kind, n], dst)

    def head(n, with_v):
        w = {"q": weight("q", n + 1), "k": weight("k", n + 1)}
        if with_v:
            w["v"] = weight("v", n)
        soon = nb if with_v else nb - 3

        def qk_steps(i):
            return [attn_step("qk", i)] + [proj_step(k, i) for k in "kq" if i >= soon]

        steps = qk_steps(nb - 1)
        if with_v:
            steps = ([proj_step("v", nb - 1)] + steps
                     + [proj_step("v", i) for i in range(nb - 1)])
        for i in reversed(range(nb)):
            steps += qk_steps(i - 1) if i > 0 else []
            steps += [attn_step("pv", i)] + [proj_step(k, i) for k in "kq" if i < soon]
        set_plan(steps)
        for (kind, i), _, _ in steps:
            if kind == "qk":
                scores(i)
            elif kind == "pv":
                values(n, i, v_s if with_v else v_early.at[n])
            else:
                project(kind, i, w[kind], {"q": q_s, "k": k_s, "v": v_s}[kind])

    def early_head(n, carry):
        @pl.when(n == 1)
        def _():
            for cp in cp_early:
                cp.wait()
            for cp in cp_main[len(cp_main) // 2:]:
                cp.start()

        head(n, False)
        return carry

    def main_heads(it, carry):
        for u in range(_UNROLL):
            head(_EARLY + it * _UNROLL + u, True)
        return carry

    lax.fori_loop(0, _EARLY, early_head, 0)
    for cp in cp_main:
        cp.wait()
    for cp in cp_late:
        cp.start()
    lax.fori_loop(0, (H - 1 - _EARLY) // _UNROLL, main_heads, 0)

    for cp in cp_late:
        cp.wait()
    wr = wr_v[...].astype(F32)
    wr = jnp.concatenate([wr[j:j + 1, :] for j in range(ncol)], axis=1)
    lane = lax.broadcasted_iota(I32, (8, 128), 1)
    router = [jnp.zeros((8, 128), F32)] * (S // 1024)

    cuts = list(range(0, S, bq)) + [S - bq // 2, S]
    chunks = list(zip(cuts, cuts[1:]))
    cp_out = [row_copy(out_v, out_hbm, out_sem.at[e], a, b - a)
              for e, (a, b) in enumerate(chunks)]

    mods = []
    c_col = jnp.broadcast_to(_rb(silu_c), (128, M)).T

    def mod_job(k):
        def job(ready):
            acc = after(jnp.zeros((8, M), F32), ready)
            for r in range(0, M, 8):
                col = after(c_col[r:r + 8], [acc[:, -128:]])
                acc = acc + (wmod_v[r:r + 8, k * M:(k + 1) * M].astype(F32)
                             * jnp.concatenate([col] * ncol, axis=1))
            mods.append(_rb(jnp.sum(acc, axis=0, keepdims=True)))
            return _vregs(acc)
        return job

    def transpose_job(src, r, c):
        def job(ready):
            w = after(pltpu.bitcast(src[r:r + 128, :], U32), ready)
            w = pltpu.bitcast(w, BF16).T
            wgu_s[:, c:c + 128] = w
            w = pltpu.bitcast(w, U32)
            return [w[j - 8:j] for j in range(64, M // 2 + 1, 64)]
        return job

    def finish_job(att, a, b, cp):
        def job(ready):
            ga, sb, cb, gb = mods
            x1b = (x_v[a:b, :].astype(F32) + _rb(ga * _rb(after(att, ready)))).astype(BF16)
            x1 = x1b.astype(F32)
            h2b = (_rb(_layernorm(x1) * _rb(1.0 + cb)) + sb).astype(BF16)
            h2 = h2b.astype(F32)
            y = x1 + _rb(gb * (h2 + h2 * 0.0))
            x1_v[a:b, :] = x1b
            h2_v[a:b, :] = h2b
            out_v[a:b, :] = y.astype(BF16)
            r = jnp.sum(h2 * wr, axis=1, keepdims=True)
            for t in range(a, b, 8):
                router[t // 1024] = jnp.where(lane == t % 1024 // 8, r[t - a:t - a + 8],
                                              router[t // 1024])
            if cp is not None:
                cp.start()
            return [router[a // 1024]] + _vregs(y)
        return job

    steps = [attn_step("qk", i) for i in range(3)]
    for i in range(nb):
        steps.append(attn_step("pv", i))
        if 0 < i < nb - 2:
            steps.append(attn_step("qk", i + 2))
        steps += [(("out", e), [b - a] * (H * ncol), range(H))
                  for e, (a, b) in enumerate(chunks) if a // bq == i]
    set_plan(steps)
    spare = [transpose_job(src, r, k * FP + r)
             for k, src in enumerate((wg_v, wu_v)) for r in range(0, FP, 128)]
    jobs = [[]] + [[mod_job(k)] for k in range(2, 6)]
    ready, due = [], []
    for (kind, i), _, _ in steps:
        if kind == "qk":
            scores(i)
        elif kind == "pv":
            values(H - 1, i, v_early.at[_EARLY])
        else:
            a, b = chunks[i]
            cols = []
            for j in range(ncol):
                results = []
                for job in jobs[j]:
                    results += job(ready)
                    ready = results[-1:]
                ctx = [ctx_s[n, a // 2:b // 2, :] for n in range(H)]
                ctx[0] = jnp.concatenate([after(ctx[0][:8], due), ctx[0][8:]], axis=0)
                ctx = planned((kind, i) if j == 0 else None, ctx)
                cols.append(jnp.dot(pltpu.bitcast(ctx, BF16), wo_v[:, j * 128:(j + 1) * 128],
                                    preferred_element_type=F32))
                ready, due = [cols[-1][-8:]], results
            att = jnp.concatenate(cols, axis=1)
            size = 16 if i < nb - 2 else 32
            todo = [finish_job(att[lo - a:lo - a + size], lo, lo + size,
                               cp_out[i] if lo + size == b else None)
                    for lo in range(a, b, size)]
            jobs = [todo[len(todo) * j // ncol:len(todo) * (j + 1) // ncol]
                    for j in range(ncol)]
            for j in range(ncol if i < nb - 2 else 0):
                if spare:
                    jobs[j].append(spare.pop(0))
    assert not spare
    finish_job(att, a, b, cp_out[-1])([])

    r = _rb(jnp.concatenate(router, axis=0))
    bits = lax.shift_right_logical(pltpu.bitcast(r, I32), 16)
    order = jnp.where(bits >= 0x8000, 0xFFFF - bits, bits + 0x8000)
    order = jnp.where(r == 0.0, 0x8000, order)
    order = jnp.where(r != r, 0, order)
    row_id = lax.broadcasted_iota(I32, r.shape, 0)
    token = ((row_id >> 3) * 1024 + (row_id & 7)
             + lax.broadcasted_iota(I32, r.shape, 1) * 8)
    key = pltpu.bitcast(0x20000000 + order * S + (S - 1 - token), F32)

    sub = lax.broadcasted_iota(I32, (16, M), 0)
    picks = []
    x_sel = jnp.zeros((16, M), F32)
    x1_sel = jnp.zeros((16, M), F32)
    r_sel = jnp.zeros((16, 1), F32)

    def picked_row(ref, base, here):
        v = jnp.where(here, ref[pl.ds(base, 16), :].astype(F32), 0.0)
        return jnp.sum(v, axis=0, keepdims=True)

    for s in range(_TOPC):
        top = jnp.max(jnp.max(key, axis=0, keepdims=True), axis=1, keepdims=True)
        hit = key == top
        key = jnp.where(hit, 0.0, key)
        r_top = jnp.sum(jnp.sum(jnp.where(hit, r, 0.0), axis=0, keepdims=True),
                        axis=1, keepdims=True)
        idx = (S - 1) - (pltpu.bitcast(top, I32)[0, 0] & (S - 1))
        picks.append((pl.multiple_of(idx & -16, 16), sub == (idx & 15)))
        x_sel = jnp.where(sub == s, picked_row(h2_v, *picks[s]), x_sel)
        x1_sel = jnp.where(sub == s, picked_row(x1_v, *picks[s]), x1_sel)
        r_sel = jnp.where(sub[:, :1] == s, r_top, r_sel)

    gu = _rb(jnp.dot(x_sel.astype(BF16), wgu_s[...], preferred_element_type=F32))
    g, u = gu[:, :FP], gu[:, FP:]
    act = (_rb(g * jax.nn.sigmoid(g)) * u).astype(BF16)
    y = _rb(jnp.dot(act, wd_v[...], preferred_element_type=F32))
    y = _rb(y * _rb(jax.nn.sigmoid(r_sel)))
    fixed = x1_sel + _rb(mods[3] * _rb(x_sel + (x_sel * 0.0 + y)))

    for cp in cp_out:
        cp.wait()
    for s, (base, here) in enumerate(picks):
        old = out_v[pl.ds(base, 16), :].astype(F32)
        out_v[pl.ds(base, 16), :] = jnp.where(here, fixed[s:s + 1, :], old).astype(BF16)

    cp_fix = [row_copy(out_v, out_hbm, fix_sem.at[s], base, 16)
              for s, (base, _) in enumerate(picks)]
    first = [True]
    for s in range(1, _TOPC):
        first.append(picks[0][0] != picks[s][0])
        for e in range(1, s):
            first[s] = jnp.logical_and(first[s], picks[e][0] != picks[s][0])
    for s in range(_TOPC):
        pl.when(first[s])(cp_fix[s].start)
    for s in range(_TOPC):
        pl.when(first[s])(cp_fix[s].wait)


@jax.jit
def pallas_adaLN_cond__compressed_kv_cla__moe_arch_mod__prompt_kernel(
    A_x: jax.Array,
    A_c_kv: jax.Array,
    A_w_q: jax.Array,
    A_w_uk: jax.Array,
    A_w_uv: jax.Array,
    A_w_o: jax.Array,
    B_x: jax.Array,
    B_w_r: jax.Array,
    B_w_gate: jax.Array,
    B_w_up: jax.Array,
    B_w_down: jax.Array,
    c: jax.Array,
    w_mod: jax.Array,
):
    del B_x
    B, S, M = A_x.shape
    DC = A_c_kv.shape[-1]
    _, H, D = A_w_q.shape
    FP = pl.cdiv(B_w_down.shape[0], 128) * 128
    assert (B, S, A_c_kv.shape[1], M, D) == (1, 2048, 2048, 640, 128)
    assert H >= 8 and H % 2 == 0 and (H - 1 - _EARLY) % _UNROLL == 0

    hbm = pl.BlockSpec(memory_space=pl.ANY)
    out = pl.pallas_call(
        _kernel,
        out_shape=jax.ShapeDtypeStruct((S, M), BF16),
        in_specs=[hbm] * 12,
        out_specs=hbm,
        scratch_shapes=[
            pltpu.VMEM((S, M), BF16),
            pltpu.VMEM((S, DC), BF16),
            pltpu.VMEM((M, 6 * M), BF16),
            pltpu.VMEM((H // 2, M + 2 * DC, D), U32),
            pltpu.VMEM((H * D, M), BF16),
            pltpu.VMEM((FP, M), BF16),
            pltpu.VMEM((FP, M), BF16),
            pltpu.VMEM((FP, M), BF16),
            pltpu.VMEM((M, 2 * FP), BF16),
            pltpu.VMEM((1, M), BF16),
            pltpu.VMEM((M // 128, 128), BF16),
            pltpu.VMEM((S // 2, M), U32),
            pltpu.VMEM((S // 2, DC), U32),
            pltpu.VMEM((S // 2, D), U32),
            pltpu.VMEM((S // 2, D), U32),
            pltpu.VMEM((S // 2, D), U32),
            pltpu.VMEM((_EARLY + 1, S // 2, D), U32),
            pltpu.VMEM((H, S // 2, D), U32),
            pltpu.VMEM((S, M), BF16),
            pltpu.VMEM((S, M), BF16),
            pltpu.VMEM((S, M), BF16),
            pltpu.VMEM((8, 128), U32),
            pltpu.SemaphoreType.DMA((14,)),
            pltpu.SemaphoreType.DMA((3 * H // 2,)),
            pltpu.SemaphoreType.DMA((S // _BQ + 1,)),
            pltpu.SemaphoreType.DMA((_TOPC,)),
        ],
        compiler_params=pltpu.CompilerParams(vmem_limit_bytes=110 * 1024 * 1024),
        name="adaln_mla_mod",
    )(
        A_x.reshape(S, M),
        A_c_kv.reshape(S, DC),
        A_w_q,
        A_w_uk,
        A_w_uv,
        A_w_o.reshape(H * D, M),
        B_w_r.reshape(M // 128, 128),
        B_w_gate.T,
        B_w_up.T,
        B_w_down,
        c,
        w_mod,
    )
    return out.reshape(B, S, M)
```
